```python
import os as _os
_os.environ.setdefault("JAX_PLATFORMS", "cpu")
import jax
import jax.numpy as jnp

def _softmax(x, axis=-1):
    return jax.nn.softmax(x, axis=axis)
def _gelu(x):
    return jax.nn.gelu(x, approximate=True)
def _silu(x):
    return jax.nn.silu(x)
def _sigmoid(x):
    return jax.nn.sigmoid(x)
def _layernorm(x, axis=-1, eps=1e-5):
    m = jnp.mean(x, axis=axis, keepdims=True)
    v = jnp.var(x, axis=axis, keepdims=True)
    return (x - m) / jnp.sqrt(v + eps)
def _scatter_add(tgt, idx, src, axis=0):
    return tgt.at[idx].add(src)
def _segment_sum(src, seg, n):
    return jax.ops.segment_sum(src, seg, n)
class _Rng:
    def __init__(self, key):
        self._k = key
    def _next(self):
        self._k, sub = jax.random.split(self._k)
        return sub
    def normal(self, shape):
        return jax.random.normal(self._next(), shape, dtype=jnp.bfloat16)
    def randint(self, lo, hi, shape):
        return jax.random.randint(self._next(), shape, lo, hi, dtype=jnp.int32)
    def uniform(self, shape, lo=0.0, hi=1.0):
        return jax.random.uniform(self._next(), shape, jnp.bfloat16, lo, hi)
    def permutation(self, n):
        return jax.random.permutation(self._next(), n)


kernel_name = 'sequential_preLN__ssm_conv_h3__mixer_s_mlp__prompt'

def setup_inputs():
    _rng = _Rng(jax.random.key(int.from_bytes(__import__("os").urandom(4), "little")))
    _w = (lambda a: (lambda t: t.astype(jnp.bfloat16) if jnp.issubdtype(t.dtype, jnp.floating) else t)(jnp.asarray(a)))
    def _A_setup():
        B, S, D = 1, 2048, 640
        ks = 4
        return {
            "q": _w((lambda *s: _rng.normal(s) * 0.05)(B, S, D)),
            "k": _w((lambda *s: _rng.normal(s) * 0.05)(B, S, D)),
            "v": _w((lambda *s: _rng.normal(s) * 0.05)(B, S, D)),
            "shift_k": _w((lambda *s: _rng.normal(s) * 0.05)(D, ks) * 0.5),
            "ssm_k": _w((lambda *s: _rng.normal(s) * 0.05)(D, S) * (1.0 / S ** 0.5)),
            "ssm_D": _w((lambda *s: _rng.normal(s) * 0.05)(D)),
        }
    _A_in = _A_setup()

    def _B_setup():
        B, S, D, F = 1, 2048, 640, 1728
        return {
            "x":  _w((lambda *s: _rng.normal(s) * 0.05)(B, S, D)),
            "w1": _w((lambda *s: _rng.normal(s) * 0.8)(D, D) * (D ** -0.5)),
            "w2": _w((lambda *s: _rng.normal(s) * 0.8)(D, D) * (D ** -0.5)),
            "w3": _w((lambda *s: _rng.normal(s) * 0.8)(D, F) * (D ** -0.5)),
            "w4": _w((lambda *s: _rng.normal(s) * 0.8)(F, D) * (F ** -0.5)),
        }
    _B_in = _B_setup()

    return {
        "A_q": _A_in["q"],
        "A_k": _A_in["k"],
        "A_v": _A_in["v"],
        "A_shift_k": _A_in["shift_k"],
        "A_ssm_k": _A_in["ssm_k"],
        "A_ssm_D": _A_in["ssm_D"],
        "B_x": _B_in["x"],
        "B_w1": _B_in["w1"],
        "B_w2": _B_in["w2"],
        "B_w3": _B_in["w3"],
        "B_w4": _B_in["w4"],
    }

def reference(A_q, A_k, A_v, A_shift_k, A_ssm_k, A_ssm_D, B_x, B_w1, B_w2, B_w3, B_w4):
    def _A_ref(q, k, v, shift_k, ssm_k, ssm_D):
        B, S, D = q.shape
        ks = shift_k.shape[-1]
        k_pad = jnp.pad(k, ((0, 0), (ks - 1, 0), (0, 0)))
        k_shift = jnp.zeros_like(k)
        for t in range(ks):
            k_shift = k_shift + k_pad[:, t:t + S, :] * shift_k[:, ks - 1 - t][None, None, :]
        kv = k_shift * v
        L = 2 * S
        kv_pad = jnp.pad(kv, ((0, 0), (0, S), (0, 0)))
        kf_pad = jnp.pad(ssm_k, ((0, 0), (0, S)))
        kv_f = (lambda x, axes=(-2,-1): jnp.fft.rfft2(x.astype(jnp.float32), axes=axes))(kv_pad[:, None, :, :], axes=(1, 2))
        kf_f = (lambda x, axes=(-2,-1): jnp.fft.rfft2(x.astype(jnp.float32), axes=axes))(kf_pad[:, None, :], axes=(1, 2))
        kf_f = (lambda x, *d: x.transpose(*d))(kf_f, 1, 2, 0)
        y_f = kv_f * kf_f[None, :, :, :]
        y = (lambda x, s, axes=(-2,-1): jnp.fft.irfft2(x, s=s, axes=axes).astype(jnp.bfloat16))(y_f, (1, L), axes=(1, 2))[:, 0, :S, :]
        y = y + kv * ssm_D[None, None, :]
        return q * y

    def _B_ref(x, w1, w2, w3, w4):
        B, S, D = x.shape
        h = _gelu(_layernorm(x, axis=-1) @ w1)
        c = D // 4
        g0 = jnp.pad(h[:, :, 0*c:1*c], ((0, 0), (1, 0), (0, 0)))[:, :S, :]
        g1 = jnp.pad(h[:, :, 1*c:2*c], ((0, 0), (0, 1), (0, 0)))[:, 1:, :]
        g2 = jnp.pad(h[:, :, 2*c:3*c], ((0, 0), (2, 0), (0, 0)))[:, :S, :]
        g3 = jnp.pad(h[:, :, 3*c:   ], ((0, 0), (0, 2), (0, 0)))[:, 2:, :]
        hs = jnp.concatenate([g0, g1, g2, g3], axis=-1) @ w2
        x1 = x + hs
        h2 = _gelu(_layernorm(x1, axis=-1) @ w3) @ w4
        return x1 + h2

    x = A_q
    h = x + _A_ref(_layernorm(x, axis=-1), A_k, A_v, A_shift_k, A_ssm_k, A_ssm_D)
    h2 = h + _B_ref(_layernorm(h, axis=-1), B_w1, B_w2, B_w3, B_w4)
    return h2
```

```python
import numpy as np
import jax
import jax.numpy as jnp
import jax.experimental.pallas as pl
import jax.experimental.pallas.tpu as pltpu

_C = 128
_EPS = 1e-5


def _dft_mats():
    c2 = 2 * _C
    k = np.arange(_C, dtype=np.float64) + 0.5
    n = np.arange(_C, dtype=np.float64)
    th = 2.0 * np.pi * np.outer(k, n) / c2
    fwd = np.concatenate([np.cos(th), -np.sin(th)], axis=0)
    n2 = np.arange(c2, dtype=np.float64)
    th2 = 2.0 * np.pi * np.outer(n2, k) / c2
    inv = np.concatenate([np.cos(th2), -np.sin(th2)], axis=1) / _C
    return fwd, inv


def _ln(x):
    m = jnp.mean(x, axis=-1, keepdims=True)
    xc = x - m
    v = jnp.mean(xc * xc, axis=-1, keepdims=True)
    return xc * jax.lax.rsqrt(v + _EPS)


def _gelu(x):
    return 0.5 * x * (1.0 + jnp.tanh(0.7978845608028654 * (x + 0.044715 * (x * x * x))))


def _kernel(q_ref, k_ref, v_ref, sk_ref, hk_ref, dd_ref, w1_ref, w2_ref, w3t_ref,
            w4_ref, f_ref, g_ref, o_ref, x_scr, h_scr, tail_scr, yprev_scr,
            hres_scr, xb_scr, h1_scr, ya_scr, *, S, D, TM):
    C = _C
    NT = S // TM
    CPT = TM // C
    bf = jnp.bfloat16
    f32 = jnp.float32
    step = pl.program_id(0)

    @pl.when(step == 0)
    def _():
        tail_scr[...] = jnp.zeros((8, D), f32)
        yprev_scr[...] = jnp.zeros((C, D), f32)
        h1_scr[0:8, :] = jnp.zeros((8, D), f32)
        h1_scr[S + 8:S + 16, :] = jnp.zeros((8, D), f32)

    @pl.when(step < NT)
    def _():
        for j in range(CPT):
            a = step * CPT + j
            g0 = pl.multiple_of(step * TM + j * C, C)
            kc = k_ref[j * C:(j + 1) * C, :].astype(f32)
            kext = jnp.concatenate([tail_scr[...], kc], axis=0)
            ks = kc * sk_ref[0:1, :]
            ks = ks + kext[7:7 + C, :] * sk_ref[1:2, :]
            ks = ks + kext[6:6 + C, :] * sk_ref[2:3, :]
            ks = ks + kext[5:5 + C, :] * sk_ref[3:4, :]
            tail_scr[...] = kc[C - 8:, :]
            kvb = (ks * v_ref[j * C:(j + 1) * C, :].astype(f32)).astype(bf)
            x_scr[a] = jnp.dot(f_ref[...], kvb, preferred_element_type=f32)
            hc = hk_ref[:, j * C:(j + 1) * C]
            h_scr[a] = jax.lax.dot_general(
                f_ref[...], hc, (((1,), (1,)), ((), ())), preferred_element_type=f32)

            RB, LB = 64, 128
            for rb in range(C // RB):
                for lb in range(D // LB):
                    rs = slice(rb * RB, (rb + 1) * RB)
                    rs2 = slice(C + rb * RB, C + (rb + 1) * RB)
                    ls = slice(lb * LB, (lb + 1) * LB)

                    def acc_body(c, acc):
                        ar, ai = acc
                        hr = h_scr[c, rs, ls]
                        hi = h_scr[c, rs2, ls]
                        xr = x_scr[a - c, rs, ls]
                        xi = x_scr[a - c, rs2, ls]
                        return (ar + hr * xr - hi * xi, ai + hr * xi + hi * xr)
                    z = jnp.zeros((RB, LB), f32)
                    ar, ai = jax.lax.fori_loop(0, a + 1, acc_body, (z, z))
                    ya_scr[rs, ls] = ar
                    ya_scr[rs2, ls] = ai
            yt = jnp.dot(g_ref[...], ya_scr[...].astype(bf), preferred_element_type=f32)
            y = yt[0:C, :] + yprev_scr[...] + kvb.astype(f32) * dd_ref[...]
            yprev_scr[...] = yt[C:2 * C, :]
            x = q_ref[j * C:(j + 1) * C, :].astype(f32)
            h = x + _ln(x) * y
            hres_scr[pl.ds(g0, C), :] = h
            xb = _ln(h)
            xb_scr[pl.ds(g0, C), :] = xb
            h1 = _gelu(jnp.dot(_ln(xb).astype(bf), w1_ref[...], preferred_element_type=f32))
            h1_scr[pl.ds(g0 + 8, C), :] = h1.astype(bf).astype(f32)

    @pl.when(step > 0)
    def _():
        cg = D // 4
        col = jax.lax.broadcasted_iota(jnp.int32, (TM, D), 1)
        r0 = pl.multiple_of((step - 1) * TM, TM)
        win = h1_scr[pl.ds(r0, TM + 16), :]
        g0 = win[7:7 + TM, :]
        g1 = win[9:9 + TM, :]
        g2 = win[6:6 + TM, :]
        g3 = win[10:10 + TM, :]
        hs = jnp.where(col < cg, g0,
                       jnp.where(col < 2 * cg, g1, jnp.where(col < 3 * cg, g2, g3)))
        x1 = xb_scr[pl.ds(r0, TM), :] + jnp.dot(hs.astype(bf), w2_ref[...],
                                                 preferred_element_type=f32)
        u = _gelu(jax.lax.dot_general(_ln(x1).astype(bf), w3t_ref[...],
                                      (((1,), (1,)), ((), ())),
                                      preferred_element_type=f32))
        h2 = jnp.dot(u.astype(bf), w4_ref[...], preferred_element_type=f32)
        o_ref[...] = (hres_scr[pl.ds(r0, TM), :] + x1 + h2).astype(o_ref.dtype)


@jax.jit
def pallas_sequential_preLN__ssm_conv_h3__mixer_s_mlp__prompt_kernel(
    A_q: jax.Array,
    A_k: jax.Array,
    A_v: jax.Array,
    A_shift_k: jax.Array,
    A_ssm_k: jax.Array,
    A_ssm_D: jax.Array,
    B_x: jax.Array,
    B_w1: jax.Array,
    B_w2: jax.Array,
    B_w3: jax.Array,
    B_w4: jax.Array,
):
    import functools
    B, S, D = A_q.shape
    F = B_w3.shape[1]
    assert B == 1 and S % _C == 0
    TM = 256
    NT = S // TM
    P = S // _C
    fwd, inv = _dft_mats()
    f_mat = jnp.asarray(fwd, dtype=jnp.bfloat16)
    g_mat = jnp.asarray(inv, dtype=jnp.bfloat16)
    q = A_q.reshape(S, D)
    k = A_k.reshape(S, D)
    v = A_v.reshape(S, D)
    sk = A_shift_k.T.astype(jnp.float32)
    dd = A_ssm_D.reshape(1, D).astype(jnp.float32)
    w3t = B_w3.T

    row = lambda i: (jnp.minimum(i, NT - 1), 0)
    const = lambda i: (0, 0)
    kern = functools.partial(_kernel, S=S, D=D, TM=TM)
    out = pl.pallas_call(
        kern,
        grid=(NT + 1,),
        in_specs=[
            pl.BlockSpec((TM, D), row),
            pl.BlockSpec((TM, D), row),
            pl.BlockSpec((TM, D), row),
            pl.BlockSpec((4, D), const),
            pl.BlockSpec((D, TM), lambda i: (0, jnp.minimum(i, NT - 1))),
            pl.BlockSpec((1, D), const),
            pl.BlockSpec((D, D), const),
            pl.BlockSpec((D, D), const),
            pl.BlockSpec((F, D), const),
            pl.BlockSpec((F, D), const),
            pl.BlockSpec((2 * _C, _C), const),
            pl.BlockSpec((2 * _C, 2 * _C), const),
        ],
        out_specs=pl.BlockSpec((TM, D), lambda i: (jnp.maximum(i - 1, 0), 0)),
        out_shape=jax.ShapeDtypeStruct((S, D), A_q.dtype),
        scratch_shapes=[
            pltpu.VMEM((P, 2 * _C, D), jnp.float32),
            pltpu.VMEM((P, 2 * _C, D), jnp.float32),
            pltpu.VMEM((8, D), jnp.float32),
            pltpu.VMEM((_C, D), jnp.float32),
            pltpu.VMEM((S, D), jnp.float32),
            pltpu.VMEM((S, D), jnp.float32),
            pltpu.VMEM((S + 16, D), jnp.float32),
            pltpu.VMEM((2 * _C, D), jnp.float32),
        ],
        compiler_params=pltpu.CompilerParams(
            dimension_semantics=("arbitrary",),
            vmem_limit_bytes=100 * 1024 * 1024),
    )(q, k, v, sk, A_ssm_k, dd, B_w1, B_w2, w3t, B_w4, f_mat, g_mat)
    return out.reshape(B, S, D)
```

```python
import numpy as np
import jax
import jax.numpy as jnp
import jax.experimental.pallas as pl
import jax.experimental.pallas.tpu as pltpu

_C = 128
_EPS = 1e-5


def _dft_mats():
    c2 = 2 * _C
    k = np.arange(_C, dtype=np.float64) + 0.5
    n = np.arange(_C, dtype=np.float64)
    th = 2.0 * np.pi * np.outer(k, n) / c2
    fwd = np.concatenate([np.cos(th), -np.sin(th)], axis=0)
    n2 = np.arange(c2, dtype=np.float64)
    th2 = 2.0 * np.pi * np.outer(n2, k) / c2
    inv = np.concatenate([np.cos(th2), -np.sin(th2)], axis=1) / _C
    return fwd, inv


def _ln(x):
    m = jnp.mean(x, axis=-1, keepdims=True)
    xc = x - m
    v = jnp.mean(xc * xc, axis=-1, keepdims=True)
    return xc * jax.lax.rsqrt(v + _EPS)


def _gelu(x):
    return 0.5 * x * (1.0 + jnp.tanh(0.7978845608028654 * (x + 0.044715 * (x * x * x))))


def _kernel(q_ref, k_ref, v_ref, sk_ref, hk_ref, dd_ref, w1_ref, w2_ref, w3t_hbm,
            w4_hbm, f_ref, g_ref, o_ref, x_scr, h_scr, tail_scr, yprev_scr,
            hres_scr, xb_scr, h1_scr, ya_scr, w3t_ref, w4_ref, wsem, *, S, D, TM):
    C = _C
    NT = S // TM
    CPT = TM // C
    bf = jnp.bfloat16
    f32 = jnp.float32
    step = pl.program_id(0)

    w3_copy = pltpu.make_async_copy(w3t_hbm, w3t_ref, wsem.at[0])
    w4_copy = pltpu.make_async_copy(w4_hbm, w4_ref, wsem.at[1])

    @pl.when(step == 0)
    def _():
        w3_copy.start()
        w4_copy.start()
        tail_scr[...] = jnp.zeros((8, D), f32)
        yprev_scr[...] = jnp.zeros((C, D), f32)
        h1_scr[0:8, :] = jnp.zeros((8, D), f32)
        h1_scr[S + 8:S + 16, :] = jnp.zeros((8, D), f32)

    @pl.when(step < NT)
    def _():
        assert CPT == 2
        a0 = step * CPT
        kvs = []
        for j in range(CPT):
            kc = k_ref[j * C:(j + 1) * C, :].astype(f32)
            kext = jnp.concatenate([tail_scr[...], kc], axis=0)
            ks = kc * sk_ref[0:1, :]
            ks = ks + kext[7:7 + C, :] * sk_ref[1:2, :]
            ks = ks + kext[6:6 + C, :] * sk_ref[2:3, :]
            ks = ks + kext[5:5 + C, :] * sk_ref[3:4, :]
            tail_scr[...] = kc[C - 8:, :]
            kvb = (ks * v_ref[j * C:(j + 1) * C, :].astype(f32)).astype(bf)
            kvs.append(kvb)
            x_scr[a0 + j] = jnp.dot(f_ref[...], kvb, preferred_element_type=f32)
            hc = hk_ref[:, j * C:(j + 1) * C]
            h_scr[a0 + j] = jax.lax.dot_general(
                f_ref[...], hc, (((1,), (1,)), ((), ())), preferred_element_type=f32)

        RB, LB = 32, 128
        for rb in range(C // RB):
            for lb in range(D // LB):
                rs = slice(rb * RB, (rb + 1) * RB)
                rs2 = slice(C + rb * RB, C + (rb + 1) * RB)
                ls = slice(lb * LB, (lb + 1) * LB)

                def acc_body(c, acc):
                    ar, ai, br, bi, pr, pi = acc
                    hr = h_scr[c, rs, ls]
                    hi = h_scr[c, rs2, ls]
                    xr = x_scr[a0 - c, rs, ls]
                    xi = x_scr[a0 - c, rs2, ls]
                    return (ar + hr * xr - hi * xi, ai + hr * xi + hi * xr,
                            br + hr * pr - hi * pi, bi + hr * pi + hi * pr, xr, xi)
                z = jnp.zeros((RB, LB), f32)
                ar, ai, br, bi, pr, pi = jax.lax.fori_loop(
                    0, a0 + 1, acc_body,
                    (z, z, z, z, x_scr[a0 + 1, rs, ls], x_scr[a0 + 1, rs2, ls]))
                hr = h_scr[a0 + 1, rs, ls]
                hi = h_scr[a0 + 1, rs2, ls]
                ya_scr[0, rs, ls] = ar
                ya_scr[0, rs2, ls] = ai
                ya_scr[1, rs, ls] = br + hr * pr - hi * pi
                ya_scr[1, rs2, ls] = bi + hr * pi + hi * pr

        for j in range(CPT):
            g0 = pl.multiple_of(step * TM + j * C, C)
            yt = jnp.dot(g_ref[...], ya_scr[j].astype(bf), preferred_element_type=f32)
            y = yt[0:C, :] + yprev_scr[...] + kvs[j].astype(f32) * dd_ref[...]
            yprev_scr[...] = yt[C:2 * C, :]
            x = q_ref[j * C:(j + 1) * C, :].astype(f32)
            h = x + _ln(x) * y
            hres_scr[pl.ds(g0, C), :] = h
            xb = _ln(h)
            xb_scr[pl.ds(g0, C), :] = xb
            h1 = _gelu(jnp.dot(_ln(xb).astype(bf), w1_ref[...], preferred_element_type=f32))
            h1_scr[pl.ds(g0 + 8, C), :] = h1.astype(bf).astype(f32)

    @pl.when(step == 1)
    def _():
        w3_copy.wait()
        w4_copy.wait()

    @pl.when(step > 0)
    def _():
        cg = D // 4
        col = jax.lax.broadcasted_iota(jnp.int32, (TM, D), 1)
        r0 = pl.multiple_of((step - 1) * TM, TM)
        win = h1_scr[pl.ds(r0, TM + 16), :]
        g0 = win[7:7 + TM, :]
        g1 = win[9:9 + TM, :]
        g2 = win[6:6 + TM, :]
        g3 = win[10:10 + TM, :]
        hs = jnp.where(col < cg, g0,
                       jnp.where(col < 2 * cg, g1, jnp.where(col < 3 * cg, g2, g3)))
        x1 = xb_scr[pl.ds(r0, TM), :] + jnp.dot(hs.astype(bf), w2_ref[...],
                                                 preferred_element_type=f32)
        u = _gelu(jax.lax.dot_general(_ln(x1).astype(bf), w3t_ref[...],
                                      (((1,), (1,)), ((), ())),
                                      preferred_element_type=f32))
        h2 = jnp.dot(u.astype(bf), w4_ref[...], preferred_element_type=f32)
        o_ref[...] = (hres_scr[pl.ds(r0, TM), :] + x1 + h2).astype(o_ref.dtype)


@jax.jit
def pallas_sequential_preLN__ssm_conv_h3__mixer_s_mlp__prompt_kernel(
    A_q: jax.Array,
    A_k: jax.Array,
    A_v: jax.Array,
    A_shift_k: jax.Array,
    A_ssm_k: jax.Array,
    A_ssm_D: jax.Array,
    B_x: jax.Array,
    B_w1: jax.Array,
    B_w2: jax.Array,
    B_w3: jax.Array,
    B_w4: jax.Array,
):
    import functools
    B, S, D = A_q.shape
    F = B_w3.shape[1]
    assert B == 1 and S % _C == 0
    TM = 256
    NT = S // TM
    P = S // _C
    fwd, inv = _dft_mats()
    f_mat = jnp.asarray(fwd, dtype=jnp.bfloat16)
    g_mat = jnp.asarray(inv, dtype=jnp.bfloat16)
    q = A_q.reshape(S, D)
    k = A_k.reshape(S, D)
    v = A_v.reshape(S, D)
    sk = A_shift_k.T.astype(jnp.float32)
    dd = A_ssm_D.reshape(1, D).astype(jnp.float32)
    w3t = B_w3.T

    row = lambda i: (jnp.minimum(i, NT - 1), 0)
    const = lambda i: (0, 0)
    kern = functools.partial(_kernel, S=S, D=D, TM=TM)
    out = pl.pallas_call(
        kern,
        grid=(NT + 1,),
        in_specs=[
            pl.BlockSpec((TM, D), row),
            pl.BlockSpec((TM, D), row),
            pl.BlockSpec((TM, D), row),
            pl.BlockSpec((4, D), const),
            pl.BlockSpec((D, TM), lambda i: (0, jnp.minimum(i, NT - 1))),
            pl.BlockSpec((1, D), const),
            pl.BlockSpec((D, D), const),
            pl.BlockSpec((D, D), const),
            pl.BlockSpec(memory_space=pl.ANY),
            pl.BlockSpec(memory_space=pl.ANY),
            pl.BlockSpec((2 * _C, _C), const),
            pl.BlockSpec((2 * _C, 2 * _C), const),
        ],
        out_specs=pl.BlockSpec((TM, D), lambda i: (jnp.maximum(i - 1, 0), 0)),
        out_shape=jax.ShapeDtypeStruct((S, D), A_q.dtype),
        scratch_shapes=[
            pltpu.VMEM((P, 2 * _C, D), jnp.float32),
            pltpu.VMEM((P, 2 * _C, D), jnp.float32),
            pltpu.VMEM((8, D), jnp.float32),
            pltpu.VMEM((_C, D), jnp.float32),
            pltpu.VMEM((S, D), jnp.float32),
            pltpu.VMEM((S, D), jnp.float32),
            pltpu.VMEM((S + 16, D), jnp.float32),
            pltpu.VMEM((2, 2 * _C, D), jnp.float32),
            pltpu.VMEM((F, D), jnp.bfloat16),
            pltpu.VMEM((F, D), jnp.bfloat16),
            pltpu.SemaphoreType.DMA((2,)),
        ],
        compiler_params=pltpu.CompilerParams(
            dimension_semantics=("arbitrary",),
            vmem_limit_bytes=100 * 1024 * 1024),
    )(q, k, v, sk, A_ssm_k, dd, B_w1, B_w2, w3t, B_w4, f_mat, g_mat)
    return out.reshape(B, S, D)
```
